```python
import os as _os
_os.environ.setdefault("JAX_PLATFORMS", "cpu")
import jax
import jax.numpy as jnp

def _softmax(x, axis=-1):
    return jax.nn.softmax(x, axis=axis)
def _gelu(x):
    return jax.nn.gelu(x, approximate=True)
def _silu(x):
    return jax.nn.silu(x)
def _sigmoid(x):
    return jax.nn.sigmoid(x)
def _layernorm(x, axis=-1, eps=1e-5):
    m = jnp.mean(x, axis=axis, keepdims=True)
    v = jnp.var(x, axis=axis, keepdims=True)
    return (x - m) / jnp.sqrt(v + eps)
def _scatter_add(tgt, idx, src, axis=0):
    return tgt.at[idx].add(src)
def _segment_sum(src, seg, n):
    return jax.ops.segment_sum(src, seg, n)
class _Rng:
    def __init__(self, key):
        self._k = key
    def _next(self):
        self._k, sub = jax.random.split(self._k)
        return sub
    def normal(self, shape):
        return jax.random.normal(self._next(), shape, dtype=jnp.bfloat16)
    def randint(self, lo, hi, shape):
        return jax.random.randint(self._next(), shape, lo, hi, dtype=jnp.int32)
    def uniform(self, shape, lo=0.0, hi=1.0):
        return jax.random.uniform(self._next(), shape, jnp.bfloat16, lo, hi)
    def permutation(self, n):
        return jax.random.permutation(self._next(), n)


kernel_name = 'interleave_layers__gqa_block_cached__dense_activation_mish__decode'

def setup_inputs():
    _rng = _Rng(jax.random.key(int.from_bytes(__import__("os").urandom(4), "little")))
    _w = (lambda a: (lambda t: t.astype(jnp.bfloat16) if jnp.issubdtype(t.dtype, jnp.floating) else t)(jnp.asarray(a)))
    def _A_setup():
        B, Sq, D = 1, 1, 512
        Hq, Hkv, Sk, Dh = 32, 8, 65536, 128
        assert Hq % Hkv == 0, (Hq, Hkv)
        return {
            "x": _w((lambda *s: _rng.normal(s) * 0.05)(B, Sq, D)),
            "k_cache": _w((lambda *s: _rng.normal(s) * 1.6)(B, Hkv, Sk, Dh)),
            "v_cache": _w((lambda *s: _rng.normal(s) * 1.6)(B, Hkv, Sk, Dh)),
            "wq": _w((lambda *s: _rng.normal(s) * 1.6)(D, Hq * Dh) * (D ** -0.5)),
            "wo": _w((lambda *s: _rng.normal(s) * 1.6)(Hq * Dh, D) * ((Hq * Dh) ** -0.5)),
        }
    _A_in = _A_setup()

    def _B_setup():
        B, S, D, F = 1, 1, 512, 1792
        return {
            "x": _w((lambda *s: _rng.normal(s) * 0.05)(B, S, D)),
            "w1": _w((lambda *s: _rng.normal(s) * 0.8)(D, F) * (D ** -0.5)),
            "b1": _w((lambda *s: _rng.normal(s) * 0.8)(F)),
            "w2": _w((lambda *s: _rng.normal(s) * 0.8)(F, D) * (F ** -0.5)),
        }
    _B_in = _B_setup()

    return {
        "A_x": _A_in["x"],
        "A_k_cache": _A_in["k_cache"],
        "A_v_cache": _A_in["v_cache"],
        "A_wq": _A_in["wq"],
        "A_wo": _A_in["wo"],
        "B_x": _B_in["x"],
        "B_w1": _B_in["w1"],
        "B_b1": _B_in["b1"],
        "B_w2": _B_in["w2"],
    }

def reference(A_x, A_k_cache, A_v_cache, A_wq, A_wo, B_x, B_w1, B_b1, B_w2):
    def _A_ref(x, k_cache, v_cache, wq, wo):
        B, Sq, D = x.shape
        Hq, Dh = 32, 128
        Hkv = k_cache.shape[1]
        rep = Hq // Hkv
        q = (lambda x, *d: x.transpose(*d))((x @ wq).reshape(B, Sq, Hq, Dh), 0, 2, 1, 3)
        k = jnp.repeat(k_cache, rep, axis=1)
        v = jnp.repeat(v_cache, rep, axis=1)
        scores = jnp.einsum("bhqd,bhkd->bhqk", q, k) * (Dh ** -0.5)
        p = _softmax(scores, axis=-1)
        o = jnp.einsum("bhqk,bhkd->bhqd", p, v)
        return (lambda x, *d: x.transpose(*d))(o, 0, 2, 1, 3).reshape(B, Sq, Hq * Dh) @ wo

    def _B_ref(x, w1, b1, w2):
        h = jnp.einsum("bsd,df->bsf", x, w1) + b1
        sp = jnp.log1p(jnp.exp(-jnp.abs(h))) + jnp.where(h > 0, h, jnp.zeros_like(h))
        act = h * jnp.tanh(sp)
        return jnp.einsum("bsf,fd->bsd", act, w2)

    x = A_x
    x = x + _A_ref(_layernorm(x, axis=-1), A_k_cache, A_v_cache, A_wq, A_wo)
    x = x + _B_ref(_layernorm(x, axis=-1), B_w1, B_b1, B_w2)
    x = x + _A_ref(_layernorm(x, axis=-1), A_k_cache, A_v_cache, A_wq, A_wo)
    x = x + _B_ref(_layernorm(x, axis=-1), B_w1, B_b1, B_w2)
    return x
```

```python
import functools

import jax
import jax.numpy as jnp
import jax.experimental.pallas as pl
import jax.experimental.pallas.tpu as pltpu


_NT = (((1,), (1,)), ((), ()))

T_CHUNK = 4096
N_SLOTS = 57
LOOKAHEAD = 4
N_SEMS = 8


def _layernorm(x, eps=1e-5):
    m = jnp.mean(x, axis=-1, keepdims=True)
    xc = x - m
    v = jnp.mean(xc * xc, axis=-1, keepdims=True)
    return xc / jnp.sqrt(v + eps)


def _kernel(x_ref, b1_ref, k_hbm, v_hbm, wq_hbm, wo_hbm, w1_hbm, w2_hbm,
            out_ref,
            kbuf, vbuf, wq_v, wo_v, w1_v, w2_v,
            q_scr, m_scr, l_scr, acc_scr, proj_scr,
            ksem, vsem, wsem,
            *, hkv, rep, dh, sk, t_chunk, n_slots, lookahead, n_sems):
    cph = sk // t_chunk
    n_chunks = hkv * cph
    n_res = min(n_slots, n_chunks)
    n_str = n_chunks - n_res
    scale = dh ** -0.5
    f32 = jnp.float32
    bf16 = jnp.bfloat16

    def kv_copies(chunk, slot, sem_idx):
        h = chunk // cph
        r0 = pl.multiple_of((chunk % cph) * t_chunk, t_chunk)
        ck = pltpu.make_async_copy(k_hbm.at[0, h, pl.ds(r0, t_chunk), :],
                                   kbuf.at[slot], ksem.at[sem_idx])
        cv = pltpu.make_async_copy(v_hbm.at[0, h, pl.ds(r0, t_chunk), :],
                                   vbuf.at[slot], vsem.at[sem_idx])
        return ck, cv

    def start_kv(chunk, slot, sem_idx):
        ck, cv = kv_copies(chunk, slot, sem_idx)
        ck.start()
        cv.start()

    def wait_kv(chunk, slot, sem_idx):
        ck, cv = kv_copies(chunk, slot, sem_idx)
        ck.wait()
        cv.wait()

    w_copies = [
        pltpu.make_async_copy(wq_hbm, wq_v, wsem.at[0]),
        pltpu.make_async_copy(wo_hbm, wo_v, wsem.at[1]),
        pltpu.make_async_copy(w1_hbm, w1_v, wsem.at[2]),
        pltpu.make_async_copy(w2_hbm, w2_v, wsem.at[3]),
    ]

    row8 = jax.lax.broadcasted_iota(jnp.int32, (8, dh), 0)

    def setup_attention(x8):
        xn = _layernorm(x8).astype(bf16)
        qf = jnp.dot(xn, wq_v[...], preferred_element_type=f32)
        for h in range(hkv):
            qh = jnp.zeros((8, dh), f32)
            for r in range(rep):
                c0 = (h * rep + r) * dh
                qh = jnp.where(row8 == r, qf[:, c0:c0 + dh], qh)
            q_scr[h] = qh.astype(bf16)
        m_scr[...] = jnp.full(m_scr.shape, -jnp.inf, f32)
        l_scr[...] = jnp.zeros(l_scr.shape, f32)
        acc_scr[...] = jnp.zeros(acc_scr.shape, f32)
        proj_scr[...] = jnp.zeros(proj_scr.shape, f32)

    def attend(chunk, slot):
        h = chunk // cph
        q = q_scr[h]
        s = jax.lax.dot_general(q, kbuf[slot], _NT,
                                preferred_element_type=f32) * scale
        m_prev = m_scr[h]
        m_new = jnp.maximum(m_prev, jnp.max(s, axis=1, keepdims=True))
        alpha = jnp.exp(m_prev - m_new)
        p = jnp.exp(s - m_new[:, :1])
        l_scr[h] = alpha * l_scr[h] + jnp.sum(p, axis=1, keepdims=True)
        pv = jnp.dot(p.astype(bf16), vbuf[slot], preferred_element_type=f32)
        acc_scr[h] = alpha * acc_scr[h] + pv
        m_scr[h] = m_new

    def project_head(h):
        o = acc_scr[h] / l_scr[h]
        lhs = jnp.concatenate(
            [jnp.where(row8 == r, o, 0.0) for r in range(rep)], axis=1)
        r0 = pl.multiple_of(h * (rep * dh), rep * dh)
        proj_scr[...] += jnp.dot(lhs.astype(bf16),
                                 wo_v[pl.ds(r0, rep * dh), :],
                                 preferred_element_type=f32)

    def finish_layer_pair(x8):
        attn = jnp.sum(proj_scr[...], axis=0, keepdims=True)
        x8 = x8 + attn
        xn = _layernorm(x8).astype(bf16)
        hh = jnp.dot(xn, w1_v[...], preferred_element_type=f32)
        hh = hh + b1_ref[...].astype(f32)
        sp = jnp.log1p(jnp.exp(-jnp.abs(hh))) + jnp.maximum(hh, 0.0)
        act = hh * jnp.tanh(sp)
        return x8 + jnp.dot(act.astype(bf16), w2_v[...],
                            preferred_element_type=f32)

    w_copies[0].start()
    for i in range(lookahead):
        start_kv(i, i % n_slots, i % n_sems)
    for c in w_copies[1:]:
        c.start()

    x8 = jnp.broadcast_to(x_ref[...].astype(f32), (8, x_ref.shape[-1]))
    w_copies[0].wait()
    setup_attention(x8)
    w_copies[1].wait()

    def pass1_body(i, carry):
        nxt = i + lookahead

        @pl.when(nxt < n_chunks)
        def _():
            start_kv(nxt, nxt % n_slots, nxt % n_sems)

        slot = i % n_slots
        wait_kv(i, slot, i % n_sems)
        attend(i, slot)

        @pl.when(i % cph == cph - 1)
        def _():
            project_head(i // cph)

        return carry

    jax.lax.fori_loop(0, n_chunks, pass1_body, 0)

    w_copies[2].wait()
    w_copies[3].wait()
    x8 = finish_layer_pair(x8)
    setup_attention(x8)

    split_head = n_str // cph if (n_str % cph != 0 or n_str == 0) else None
    if n_str == 0:
        split_head = None

    def maybe_project(chunk):
        cond = chunk % cph == cph - 1
        if split_head is not None:
            cond = jnp.logical_and(cond, chunk // cph != split_head)

        @pl.when(cond)
        def _():
            project_head(chunk // cph)

    n_a = min(lookahead, n_res)

    def str_slot(i):
        return (n_str + (i % n_a)) % n_slots

    for i in range(n_a):
        c = n_str + i
        attend(c, c % n_slots)
        if i < n_str:
            start_kv(i, c % n_slots, i % n_sems)
        if c % cph == cph - 1 and c // cph != split_head:
            project_head(c // cph)

    n_iter = max(n_str, n_res - n_a)

    def pass2_body(i, carry):
        @pl.when(i < n_res - n_a)
        def _():
            c = n_str + n_a + i
            attend(c, c % n_slots)
            maybe_project(c)

        @pl.when(i < n_str)
        def _():
            slot = str_slot(i)
            wait_kv(i, slot, i % n_sems)
            attend(i, slot)

            @pl.when(i + n_a < n_str)
            def _():
                start_kv(i + n_a, slot, (i + n_a) % n_sems)

            maybe_project(i)

        return carry

    jax.lax.fori_loop(0, n_iter, pass2_body, 0)
    if split_head is not None:
        project_head(split_head)

    x8 = finish_layer_pair(x8)
    out_ref[...] = x8[0:1, :].astype(out_ref.dtype)


@jax.jit
def pallas_interleave_layers__gqa_block_cached__dense_activation_mish__decode_kernel(
    A_x: jax.Array,
    A_k_cache: jax.Array,
    A_v_cache: jax.Array,
    A_wq: jax.Array,
    A_wo: jax.Array,
    B_x: jax.Array,
    B_w1: jax.Array,
    B_b1: jax.Array,
    B_w2: jax.Array,
):
    del B_x
    B, Sq, D = A_x.shape
    assert B == 1 and Sq == 1
    _, hkv, sk, dh = A_k_cache.shape
    hq = A_wq.shape[1] // dh
    rep = hq // hkv
    F = B_w1.shape[1]
    assert rep <= 8 and sk % T_CHUNK == 0

    x2 = A_x.reshape(1, D)
    b1 = B_b1.reshape(1, F)

    kernel = functools.partial(
        _kernel, hkv=hkv, rep=rep, dh=dh, sk=sk, t_chunk=T_CHUNK,
        n_slots=N_SLOTS, lookahead=LOOKAHEAD, n_sems=N_SEMS)

    vmem = pl.BlockSpec(memory_space=pltpu.VMEM)
    hbm = pl.BlockSpec(memory_space=pl.ANY)
    out = pl.pallas_call(
        kernel,
        out_shape=jax.ShapeDtypeStruct((1, D), A_x.dtype),
        in_specs=[vmem, vmem, hbm, hbm, hbm, hbm, hbm, hbm],
        out_specs=vmem,
        scratch_shapes=[
            pltpu.VMEM((N_SLOTS, T_CHUNK, dh), A_k_cache.dtype),
            pltpu.VMEM((N_SLOTS, T_CHUNK, dh), A_v_cache.dtype),
            pltpu.VMEM(A_wq.shape, A_wq.dtype),
            pltpu.VMEM(A_wo.shape, A_wo.dtype),
            pltpu.VMEM(B_w1.shape, B_w1.dtype),
            pltpu.VMEM(B_w2.shape, B_w2.dtype),
            pltpu.VMEM((hkv, 8, dh), jnp.bfloat16),
            pltpu.VMEM((hkv, 8, dh), jnp.float32),
            pltpu.VMEM((hkv, 8, dh), jnp.float32),
            pltpu.VMEM((hkv, 8, dh), jnp.float32),
            pltpu.VMEM((8, D), jnp.float32),
            pltpu.SemaphoreType.DMA((N_SEMS,)),
            pltpu.SemaphoreType.DMA((N_SEMS,)),
            pltpu.SemaphoreType.DMA((4,)),
        ],
        compiler_params=pltpu.CompilerParams(
            vmem_limit_bytes=128 * 1024 * 1024),
    )(x2, b1, A_k_cache, A_v_cache, A_wq, A_wo, B_w1, B_w2)
    return out.reshape(B, Sq, D)
```

```python
import functools

import jax
import jax.numpy as jnp
import jax.experimental.pallas as pl
import jax.experimental.pallas.tpu as pltpu


_NT = (((1,), (1,)), ((), ()))

T_CHUNK = 2048
N_SLOTS = 116
LOOKAHEAD = 4
N_SEMS = 8


def _layernorm(x, eps=1e-5):
    m = jnp.mean(x, axis=-1, keepdims=True)
    xc = x - m
    v = jnp.mean(xc * xc, axis=-1, keepdims=True)
    return xc / jnp.sqrt(v + eps)


def _kernel(x_hbm, b1_hbm, k_hbm, v_hbm, wq_hbm, wo_hbm, w1_hbm, w2_hbm,
            out_ref,
            kbuf, vbuf, wq_v, wo_v, w1_v, w2_v, x_v, b1_v,
            q_scr, m_scr, l_scr, acc_scr, proj_scr,
            ksem, vsem, wsem,
            *, hkv, rep, dh, sk, t_chunk, n_slots, lookahead, n_sems):
    cph = sk // t_chunk
    n_chunks = hkv * cph
    n_res = min(n_slots, n_chunks)
    n_str = n_chunks - n_res
    scale = dh ** -0.5
    f32 = jnp.float32
    bf16 = jnp.bfloat16
    d_model = x_v.shape[-1]

    def k_copy(chunk, slot, sem_idx):
        h = chunk // cph
        r0 = pl.multiple_of((chunk % cph) * t_chunk, t_chunk)
        return pltpu.make_async_copy(k_hbm.at[0, h, pl.ds(r0, t_chunk), :],
                                     kbuf.at[slot], ksem.at[sem_idx])

    def v_copy(chunk, slot, sem_idx):
        h = chunk // cph
        r0 = pl.multiple_of((chunk % cph) * t_chunk, t_chunk)
        return pltpu.make_async_copy(v_hbm.at[0, h, pl.ds(r0, t_chunk), :],
                                     vbuf.at[slot], vsem.at[sem_idx])

    def start_kv(chunk, slot, sem_idx):
        k_copy(chunk, slot, sem_idx).start()
        v_copy(chunk, slot, sem_idx).start()

    cp_x = pltpu.make_async_copy(x_hbm, x_v, wsem.at[0])
    cp_wq = pltpu.make_async_copy(wq_hbm, wq_v, wsem.at[1])
    cp_wo = pltpu.make_async_copy(wo_hbm, wo_v, wsem.at[2])
    cp_w1 = pltpu.make_async_copy(w1_hbm, w1_v, wsem.at[3])
    cp_b1 = pltpu.make_async_copy(b1_hbm, b1_v, wsem.at[4])
    cp_w2 = pltpu.make_async_copy(w2_hbm, w2_v, wsem.at[5])

    row8 = jax.lax.broadcasted_iota(jnp.int32, (8, dh), 0)

    def reset_state():
        m_scr[...] = jnp.full(m_scr.shape, -jnp.inf, f32)
        l_scr[...] = jnp.zeros(l_scr.shape, f32)
        acc_scr[...] = jnp.zeros(acc_scr.shape, f32)
        proj_scr[...] = jnp.zeros(proj_scr.shape, f32)

    def q_heads(xn, heads):
        for h in heads:
            c0 = h * rep * dh
            qf = jnp.dot(xn, wq_v[:, c0:c0 + rep * dh],
                         preferred_element_type=f32)
            qh = jnp.zeros((8, dh), f32)
            for r in range(rep):
                qh = jnp.where(row8 == r, qf[:, r * dh:(r + 1) * dh], qh)
            q_scr[h] = qh.astype(bf16)

    def attend(chunk, slot, after_k=None, before_v=None):
        h = chunk // cph
        q = q_scr[h]
        s = jax.lax.dot_general(q, kbuf[slot], _NT,
                                preferred_element_type=f32) * scale
        if after_k is not None:
            after_k()
        m_prev = m_scr[h]
        m_new = jnp.maximum(m_prev, jnp.max(s, axis=1, keepdims=True))
        alpha = jnp.exp(m_prev - m_new)
        p = jnp.exp(s - m_new[:, :1])
        l_scr[h] = alpha * l_scr[h] + jnp.sum(p, axis=1, keepdims=True)
        m_scr[h] = m_new
        if before_v is not None:
            before_v()
        pv = jnp.dot(p.astype(bf16), vbuf[slot], preferred_element_type=f32)
        acc_scr[h] = alpha * acc_scr[h] + pv

    def attend_streamed(chunk, slot, sem_idx):
        k_copy(chunk, slot, sem_idx).wait()
        attend(chunk, slot,
               before_v=lambda: v_copy(chunk, slot, sem_idx).wait())

    def project_head(h):
        o = acc_scr[h] / l_scr[h]
        lhs = jnp.concatenate(
            [jnp.where(row8 == r, o, 0.0) for r in range(rep)], axis=1)
        r0 = pl.multiple_of(h * (rep * dh), rep * dh)
        proj_scr[...] += jnp.dot(lhs.astype(bf16),
                                 wo_v[pl.ds(r0, rep * dh), :],
                                 preferred_element_type=f32)

    def finish_layer_pair(x8):
        attn = jnp.sum(proj_scr[...], axis=0, keepdims=True)
        x8 = x8 + attn
        xn = _layernorm(x8).astype(bf16)
        hh = jnp.dot(xn, w1_v[...], preferred_element_type=f32)
        hh = hh + b1_v[...].astype(f32).reshape(1, -1)
        sp = jnp.log1p(jnp.exp(-jnp.abs(hh))) + jnp.maximum(hh, 0.0)
        act = hh * jnp.tanh(sp)
        return x8 + jnp.dot(act.astype(bf16), w2_v[...],
                            preferred_element_type=f32)

    cp_wq.start()
    cp_x.start()
    for i in range(lookahead):
        start_kv(i, i % n_slots, i % n_sems)
    cp_wo.start()
    cp_w1.start()
    cp_b1.start()
    cp_w2.start()

    reset_state()
    cp_x.wait()
    x8 = jnp.broadcast_to(x_v[0].astype(f32), (8, d_model))
    xn = _layernorm(x8).astype(bf16)
    cp_wq.wait()
    q_heads(xn, range(hkv))

    def pass1_body(i, carry):
        nxt = i + lookahead

        @pl.when(nxt < n_chunks)
        def _():
            start_kv(nxt, nxt % n_slots, nxt % n_sems)

        attend_streamed(i, i % n_slots, i % n_sems)

        @pl.when(i == cph - 1)
        def _():
            cp_wo.wait()

        @pl.when(i % cph == cph - 1)
        def _():
            project_head(i // cph)

        return carry

    jax.lax.fori_loop(0, n_chunks, pass1_body, 0)

    cp_w1.wait()
    cp_b1.wait()
    cp_w2.wait()
    x8 = finish_layer_pair(x8)
    reset_state()
    xn = _layernorm(x8).astype(bf16)

    split_head = n_str // cph if n_str % cph != 0 else None

    def maybe_project(chunk):
        cond = chunk % cph == cph - 1
        if split_head is not None:
            cond = jnp.logical_and(cond, chunk // cph != split_head)

        @pl.when(cond)
        def _():
            project_head(chunk // cph)

    n_a = min(lookahead, n_res)

    def str_slot(i):
        return (n_str + (i % n_a)) % n_slots

    q_done = set()
    for i in range(n_a):
        c = n_str + i
        slot = c % n_slots
        need = [c // cph] if i < 2 else list(range(hkv))
        q_heads(xn, [h for h in need if h not in q_done])
        q_done.update(need)
        if i < n_str:
            attend(c, slot,
                   after_k=lambda: k_copy(i, slot, i % n_sems).start())
            v_copy(i, slot, i % n_sems).start()
        else:
            attend(c, slot)
        if c % cph == cph - 1 and c // cph != split_head:
            project_head(c // cph)
    q_heads(xn, [h for h in range(hkv) if h not in q_done])

    n_iter = max(n_str, n_res - n_a)

    def pass2_body(i, carry):
        @pl.when(i < n_res - n_a)
        def _():
            c = n_str + n_a + i
            attend(c, c % n_slots)
            maybe_project(c)

        @pl.when(i < n_str)
        def _():
            slot = str_slot(i)
            attend_streamed(i, slot, i % n_sems)

            @pl.when(i + n_a < n_str)
            def _():
                start_kv(i + n_a, slot, (i + n_a) % n_sems)

            maybe_project(i)

        return carry

    jax.lax.fori_loop(0, n_iter, pass2_body, 0)
    if split_head is not None:
        project_head(split_head)

    x8 = finish_layer_pair(x8)
    out_ref[0] = x8[0:1, :].astype(out_ref.dtype)


@jax.jit
def pallas_interleave_layers__gqa_block_cached__dense_activation_mish__decode_kernel(
    A_x: jax.Array,
    A_k_cache: jax.Array,
    A_v_cache: jax.Array,
    A_wq: jax.Array,
    A_wo: jax.Array,
    B_x: jax.Array,
    B_w1: jax.Array,
    B_b1: jax.Array,
    B_w2: jax.Array,
):
    del B_x
    B, Sq, D = A_x.shape
    assert B == 1 and Sq == 1
    _, hkv, sk, dh = A_k_cache.shape
    hq = A_wq.shape[1] // dh
    rep = hq // hkv
    assert rep <= 8 and sk % T_CHUNK == 0

    kernel = functools.partial(
        _kernel, hkv=hkv, rep=rep, dh=dh, sk=sk, t_chunk=T_CHUNK,
        n_slots=N_SLOTS, lookahead=LOOKAHEAD, n_sems=N_SEMS)

    hbm = pl.BlockSpec(memory_space=pl.ANY)
    return pl.pallas_call(
        kernel,
        out_shape=jax.ShapeDtypeStruct((B, Sq, D), A_x.dtype),
        in_specs=[hbm] * 8,
        out_specs=pl.BlockSpec(memory_space=pltpu.VMEM),
        scratch_shapes=[
            pltpu.VMEM((N_SLOTS, T_CHUNK, dh), A_k_cache.dtype),
            pltpu.VMEM((N_SLOTS, T_CHUNK, dh), A_v_cache.dtype),
            pltpu.VMEM(A_wq.shape, A_wq.dtype),
            pltpu.VMEM(A_wo.shape, A_wo.dtype),
            pltpu.VMEM(B_w1.shape, B_w1.dtype),
            pltpu.VMEM(B_w2.shape, B_w2.dtype),
            pltpu.VMEM(A_x.shape, A_x.dtype),
            pltpu.VMEM(B_b1.shape, B_b1.dtype),
            pltpu.VMEM((hkv, 8, dh), jnp.bfloat16),
            pltpu.VMEM((hkv, 8, dh), jnp.float32),
            pltpu.VMEM((hkv, 8, dh), jnp.float32),
            pltpu.VMEM((hkv, 8, dh), jnp.float32),
            pltpu.VMEM((8, D), jnp.float32),
            pltpu.SemaphoreType.DMA((N_SEMS,)),
            pltpu.SemaphoreType.DMA((N_SEMS,)),
            pltpu.SemaphoreType.DMA((6,)),
        ],
        compiler_params=pltpu.CompilerParams(
            vmem_limit_bytes=128 * 1024 * 1024),
    )(A_x, B_b1, A_k_cache, A_v_cache, A_wq, A_wo, B_w1, B_w2)
```
